```python
import os as _os
_os.environ.setdefault("JAX_PLATFORMS", "cpu")
import jax
import jax.numpy as jnp

def _softmax(x, axis=-1):
    return jax.nn.softmax(x, axis=axis)
def _gelu(x):
    return jax.nn.gelu(x, approximate=True)
def _silu(x):
    return jax.nn.silu(x)
def _sigmoid(x):
    return jax.nn.sigmoid(x)
def _layernorm(x, axis=-1, eps=1e-5):
    m = jnp.mean(x, axis=axis, keepdims=True)
    v = jnp.var(x, axis=axis, keepdims=True)
    return (x - m) / jnp.sqrt(v + eps)
def _scatter_add(tgt, idx, src, axis=0):
    return tgt.at[idx].add(src)
def _segment_sum(src, seg, n):
    return jax.ops.segment_sum(src, seg, n)
class _Rng:
    def __init__(self, key):
        self._k = key
    def _next(self):
        self._k, sub = jax.random.split(self._k)
        return sub
    def normal(self, shape):
        return jax.random.normal(self._next(), shape, dtype=jnp.bfloat16)
    def randint(self, lo, hi, shape):
        return jax.random.randint(self._next(), shape, lo, hi, dtype=jnp.int32)
    def uniform(self, shape, lo=0.0, hi=1.0):
        return jax.random.uniform(self._next(), shape, jnp.bfloat16, lo, hi)
    def permutation(self, n):
        return jax.random.permutation(self._next(), n)


kernel_name = 'standalone__gqa_block_cached__near_ridge'

def setup_inputs():
    _rng = _Rng(jax.random.key(int.from_bytes(__import__("os").urandom(4), "little")))
    _w = (lambda a: (lambda t: t.astype(jnp.bfloat16) if jnp.issubdtype(t.dtype, jnp.floating) else t)(jnp.asarray(a)))
    B, Sq, D = 8, 96, 448
    Hq, Hkv, Sk, Dh = 16, 8, 2048, 256
    assert Hq % Hkv == 0, (Hq, Hkv)
    return {
        "x": _w((lambda *s: _rng.normal(s) * 0.8)(B, Sq, D)),
        "k_cache": _w((lambda *s: _rng.normal(s) * 0.8)(B, Hkv, Sk, Dh)),
        "v_cache": _w((lambda *s: _rng.normal(s) * 0.05)(B, Hkv, Sk, Dh)),
        "wq": _w((lambda *s: _rng.normal(s) * 0.8)(D, Hq * Dh) * (D ** -0.5)),
        "wo": _w((lambda *s: _rng.normal(s) * 0.05)(Hq * Dh, D) * ((Hq * Dh) ** -0.5)),
    }

def reference(x, k_cache, v_cache, wq, wo):
    B, Sq, D = x.shape
    Hq, Dh = 16, 256
    Hkv = k_cache.shape[1]
    rep = Hq // Hkv
    q = (lambda x, *d: x.transpose(*d))((x @ wq).reshape(B, Sq, Hq, Dh), 0, 2, 1, 3)
    k = jnp.repeat(k_cache, rep, axis=1)
    v = jnp.repeat(v_cache, rep, axis=1)
    scores = jnp.einsum("bhqd,bhkd->bhqk", q, k) * (Dh ** -0.5)
    p = _softmax(scores, axis=-1)
    o = jnp.einsum("bhqk,bhkd->bhqd", p, v)
    return (lambda x, *d: x.transpose(*d))(o, 0, 2, 1, 3).reshape(B, Sq, Hq * Dh) @ wo
```

```python
import math

import jax
import jax.numpy as jnp
from jax import lax
import jax.experimental.pallas as pl
import jax.experimental.pallas.tpu as pltpu

_HQ, _DH = 16, 256
_NB = 3
_CK = 512
_ORDER = "V0_K0_E0_V1_K1_E1_V2_K2_E2_V3_K3_E3_F_Q_O".split("_")


@jax.jit
def pallas_standalone__gqa_block_cached__near_ridge_kernel(
    x: jax.Array,
    k_cache: jax.Array,
    v_cache: jax.Array,
    wq: jax.Array,
    wo: jax.Array,
):
    B, Sq, D = x.shape
    _, Hkv, Sk, Dh = k_cache.shape
    rep = _HQ // Hkv
    assert Dh == _DH and rep == 2 and Sk % _CK == 0 and Sk // _CK == 4
    W = rep * Dh
    NS = B * Hkv
    NC = Sk // _CK
    nb, ck = _NB, _CK
    C = (Dh ** -0.5) * math.log2(math.e)
    f32, bf16 = jnp.float32, jnp.bfloat16
    NT = (((1,), (1,)), ((), ()))

    def kernel(x_hbm, wq_hbm, k_hbm, v_hbm, woT_hbm, out_hbm,
               xb, wqb, wob, kbuf, vbuf, q_scr, p_scr, a_scr, o_scr, acc, outb,
               ksem, vsem, wqsem, wosem, osem, xsem):
        def kcopy(s, slot):
            return pltpu.make_async_copy(k_hbm.at[s % B, s // B], kbuf.at[slot], ksem.at[slot])

        def vcopy(s, slot):
            return pltpu.make_async_copy(v_hbm.at[s % B, s // B], vbuf.at[slot], vsem.at[slot])

        def wqcopy(h):
            return pltpu.make_async_copy(
                wq_hbm.at[:, pl.ds(pl.multiple_of(h * W, W), W)], wqb.at[h], wqsem.at[h])

        def wocopy(h):
            return pltpu.make_async_copy(
                woT_hbm.at[:, pl.ds(pl.multiple_of(h * W, W), W)], wob.at[h], wosem.at[h])

        def ocopy(b):
            return pltpu.make_async_copy(outb.at[b], out_hbm.at[b], osem.at[b])

        def qproj(s):
            q = jnp.dot(xb[s % B], wqb[s // B], preferred_element_type=f32)
            q = (q * C).astype(bf16)
            q_scr[0:Sq, :] = q[:, :Dh]
            q_scr[Sq:2 * Sq, :] = q[:, Dh:]

        def run(seq, s, kslot, vslot):
            st = {}
            for it in seq:
                j = int(it[1:]) if len(it) > 1 else None
                if it[0] == "K":
                    if "q" not in st:
                        st["q"] = q_scr[...]
                    sj = lax.dot_general(st["q"], kbuf[kslot, j * ck:(j + 1) * ck, :], NT,
                                         preferred_element_type=f32)
                    st["s", j] = sj
                    mj = sj[:, 0:128]
                    for t in range(1, ck // 128):
                        mj = jnp.maximum(mj, sj[:, t * 128:(t + 1) * 128])
                    st["m", j] = jnp.max(mj, axis=-1, keepdims=True)
                elif it[0] == "E":
                    p = jnp.exp2(st.pop(("s", j)) - st["m", j])
                    lj = p[:, 0:128]
                    for t in range(1, ck // 128):
                        lj = lj + p[:, t * 128:(t + 1) * 128]
                    st["l", j] = jnp.sum(lj, axis=-1, keepdims=True)
                    st["p", j] = p.astype(bf16)
                    if ("v", j) in st:
                        p_scr[:, j * ck:(j + 1) * ck] = st.pop(("p", j))
                    st["ne"] = st.get("ne", 0) + 1
                    if st["ne"] == NC:
                        m = st["m", 0]
                        for t in range(1, NC):
                            m = jnp.maximum(m, st["m", t])
                        al = [jnp.exp2(st["m", t] - m) for t in range(NC)]
                        l = al[0] * st["l", 0]
                        for t in range(1, NC):
                            l = l + al[t] * st["l", t]
                        r = 1.0 / l
                        st["anew"] = [a * r for a in al]
                elif it[0] == "V":
                    oj = jnp.dot(p_scr[:, j * ck:(j + 1) * ck], vbuf[vslot, j * ck:(j + 1) * ck, :],
                                 preferred_element_type=f32)
                    oj = oj * a_scr[j, :, 0:1]
                    st["o"] = oj if "o" not in st else st["o"] + oj
                    st["v", j] = True
                elif it[0] == "F":
                    o = st["o"].astype(bf16)
                    o_scr[:, 0:Dh] = o[:Sq]
                    o_scr[:, Dh:2 * Dh] = o[Sq:]
                elif it[0] == "O":
                    c = lax.dot_general(o_scr[...], wob[s // B], NT, preferred_element_type=f32)
                    c = acc[s % B] + c
                    acc[s % B] = c
                    outb[s % B] = c.astype(bf16)
                elif it[0] == "Q":
                    qproj(jnp.minimum(s + 2, NS - 1))
            for j in range(NC):
                if ("p", j) in st:
                    p_scr[:, j * ck:(j + 1) * ck] = st.pop(("p", j))
            if "anew" in st:
                for t in range(NC):
                    a_scr[t] = jnp.broadcast_to(st["anew"][t], (2 * Sq, 128))

        xcopy = pltpu.make_async_copy(x_hbm, xb, xsem.at[0])
        xcopy.start()
        wqcopy(0).start()
        kcopy(0, 0).start()
        kcopy(1, 1).start()
        vcopy(0, 0).start()
        wocopy(0).start()
        for s0 in range(2, nb):
            kcopy(s0, s0).start()
        for s0 in range(1, nb):
            vcopy(s0, s0).start()
        acc[...] = jnp.zeros_like(acc)
        xcopy.wait()
        wqcopy(0).wait()
        qproj(0)
        kcopy(0, 0).wait()
        run([f"K{j}" for j in range(NC)] + [f"E{j}" for j in range(NC)], -1, 0, 0)
        qproj(1)
        kcopy(nb, 0).start()
        wocopy(0).wait()

        def body(s, carry):
            vslot, kslot = carry
            h = s // B
            b = s % B
            more = h + 1 < Hkv

            @pl.when(jnp.logical_and(more, b == 1))
            def _():
                wqcopy(h + 1).start()

            @pl.when(jnp.logical_and(more, b == 2))
            def _():
                wocopy(h + 1).start()

            @pl.when(jnp.logical_and(more, b == B - 2))
            def _():
                wqcopy(h + 1).wait()

            @pl.when(jnp.logical_and(h > 0, b == 0))
            def _():
                wocopy(h).wait()

            kcopy(s + 1, kslot).wait()
            vcopy(s, vslot).wait()
            run(_ORDER, s, kslot, vslot)

            @pl.when(s + 1 + nb < NS)
            def _():
                kcopy(s + 1 + nb, kslot).start()

            @pl.when(s + nb < NS)
            def _():
                vcopy(s + nb, vslot).start()

            v2 = vslot + 1
            k2 = kslot + 1
            return jnp.where(v2 == nb, 0, v2), jnp.where(k2 == nb, 0, k2)

        lax.fori_loop(0, NS - 1, body, (jnp.int32(0), jnp.int32(1 % nb)))

        for b0 in range(B - 1):
            ocopy(b0).start()
        ls = (NS - 1) % nb
        vcopy(NS - 1, ls).wait()
        run([f"V{j}" for j in range(NC)] + ["F", "O"], NS - 1, 0, ls)
        ocopy(B - 1).start()
        for b0 in range(B):
            ocopy(b0).wait()

    hbm = pl.BlockSpec(memory_space=pl.ANY)
    return pl.pallas_call(
        kernel,
        in_specs=[hbm] * 5,
        out_specs=hbm,
        out_shape=jax.ShapeDtypeStruct((B, Sq, D), bf16),
        scratch_shapes=[
            pltpu.VMEM((B, Sq, D), bf16),
            pltpu.VMEM((Hkv, D, W), bf16),
            pltpu.VMEM((Hkv, D, W), bf16),
            pltpu.VMEM((nb, Sk, Dh), bf16),
            pltpu.VMEM((nb, Sk, Dh), bf16),
            pltpu.VMEM((2 * Sq, Dh), bf16),
            pltpu.VMEM((2 * Sq, Sk), bf16),
            pltpu.VMEM((NC, 2 * Sq, 128), f32),
            pltpu.VMEM((Sq, W), bf16),
            pltpu.VMEM((B, Sq, D), f32),
            pltpu.VMEM((B, Sq, D), bf16),
            pltpu.SemaphoreType.DMA((nb,)),
            pltpu.SemaphoreType.DMA((nb,)),
            pltpu.SemaphoreType.DMA((Hkv,)),
            pltpu.SemaphoreType.DMA((Hkv,)),
            pltpu.SemaphoreType.DMA((B,)),
            pltpu.SemaphoreType.DMA((1,)),
        ],
        compiler_params=pltpu.CompilerParams(
            vmem_limit_bytes=100 * 1024 * 1024, disable_bounds_checks=True),
    )(x, wq, k_cache, v_cache, wo.T)
```
